```python
import os as _os
_os.environ.setdefault("JAX_PLATFORMS", "cpu")
import jax
import jax.numpy as jnp

def _softmax(x, axis=-1):
    return jax.nn.softmax(x, axis=axis)
def _gelu(x):
    return jax.nn.gelu(x, approximate=True)
def _silu(x):
    return jax.nn.silu(x)
def _sigmoid(x):
    return jax.nn.sigmoid(x)
def _layernorm(x, axis=-1, eps=1e-5):
    m = jnp.mean(x, axis=axis, keepdims=True)
    v = jnp.var(x, axis=axis, keepdims=True)
    return (x - m) / jnp.sqrt(v + eps)
def _scatter_add(tgt, idx, src, axis=0):
    return tgt.at[idx].add(src)
def _segment_sum(src, seg, n):
    return jax.ops.segment_sum(src, seg, n)
class _Rng:
    def __init__(self, key):
        self._k = key
    def _next(self):
        self._k, sub = jax.random.split(self._k)
        return sub
    def normal(self, shape):
        return jax.random.normal(self._next(), shape, dtype=jnp.bfloat16)
    def randint(self, lo, hi, shape):
        return jax.random.randint(self._next(), shape, lo, hi, dtype=jnp.int32)
    def uniform(self, shape, lo=0.0, hi=1.0):
        return jax.random.uniform(self._next(), shape, jnp.bfloat16, lo, hi)
    def permutation(self, n):
        return jax.random.permutation(self._next(), n)


kernel_name = 'gated_mix__grouped_kv_mqa__glu_gated_reglu__prompt'

def setup_inputs():
    _rng = _Rng(jax.random.key(int.from_bytes(__import__("os").urandom(4), "little")))
    _w = (lambda a: (lambda t: t.astype(jnp.bfloat16) if jnp.issubdtype(t.dtype, jnp.floating) else t)(jnp.asarray(a)))
    def _A_setup():
        B, S, D, H = 1, 2048, 1024, 32
        Dh = D // H
        return {
            "x": _w((lambda *s: _rng.normal(s) * 0.05)(B, S, D)),
            "wq": _w((lambda *s: _rng.normal(s) * 0.2)(D, H * Dh)),
            "wk": _w((lambda *s: _rng.normal(s) * 0.2)(D, Dh)),
            "wv": _w((lambda *s: _rng.normal(s) * 0.05)(D, Dh)),
            "wo": _w((lambda *s: _rng.normal(s) * 0.05)(H * Dh, D)),
        }
    _A_in = _A_setup()

    def _B_setup():
        B, S, D, F = 1, 2048, 1024, 3584
        return {
            "x": _w((lambda *s: _rng.normal(s) * 0.05)(B, S, D)),
            "W_gate": _w((lambda *s: _rng.normal(s) * 0.8)(D, F) * (2.0 / D) ** 0.5),
            "W_up": _w((lambda *s: _rng.normal(s) * 0.8)(D, F) * (2.0 / D) ** 0.5),
            "W_down": _w((lambda *s: _rng.normal(s) * 0.8)(F, D) * (1.0 / F) ** 0.5),
        }
    _B_in = _B_setup()

    return {
        "A_x": _A_in["x"],
        "A_wq": _A_in["wq"],
        "A_wk": _A_in["wk"],
        "A_wv": _A_in["wv"],
        "A_wo": _A_in["wo"],
        "B_x": _B_in["x"],
        "B_W_gate": _B_in["W_gate"],
        "B_W_up": _B_in["W_up"],
        "B_W_down": _B_in["W_down"],
        "gate_w": _w((lambda *s: _rng.normal(s) * 0.05)(1024) * 16.0),
    }

def reference(A_x, A_wq, A_wk, A_wv, A_wo, B_x, B_W_gate, B_W_up, B_W_down, gate_w):
    def _A_ref(x, wq, wk, wv, wo):
        B, S, D = x.shape
        H = 32
        Dh = D // H
        q = (lambda x, *d: x.transpose(*d))((x @ wq).reshape(B, S, H, Dh), 0, 2, 1, 3)
        k = x @ wk
        v = x @ wv
        scores = jnp.einsum("bhqd,bkd->bhqk", q, k) * (Dh ** -0.5)
        p = _softmax(scores, axis=-1)
        o = jnp.einsum("bhqk,bkd->bhqd", p, v)
        return (lambda x, *d: x.transpose(*d))(o, 0, 2, 1, 3).reshape(B, S, H * Dh) @ wo

    def _B_ref(x, W_gate, W_up, W_down):
        gate = jnp.einsum("bsd,df->bsf", x, W_gate)
        up = jnp.einsum("bsd,df->bsf", x, W_up)
        gate = gate * (lambda x, dt: x.astype(dt))(gate > 0, gate.dtype)
        h = gate * up
        return jnp.einsum("bsf,fd->bsd", h, W_down)

    x = A_x
    g = _sigmoid((x * gate_w).sum(-1, keepdims=True))
    a = _A_ref(x, A_wq, A_wk, A_wv, A_wo)
    b = _B_ref(x, B_W_gate, B_W_up, B_W_down)
    return g * a + (1 - g) * b
```

```python
import functools
import math

import jax
import jax.numpy as jnp
from jax import lax
from jax.experimental import pallas as pl
from jax.experimental.pallas import tpu as pltpu

BF = jnp.bfloat16
F32 = jnp.float32
U32 = jnp.uint32
NT = (((1,), (1,)), ((), ()))


def _bf(x):
    return pltpu.bitcast(x, BF)


def _u32(x):
    return pltpu.bitcast(x, U32)


def _tree(op, xs):
    xs = list(xs)
    while len(xs) > 1:
        xs = [op(xs[i], xs[i + 1]) if i + 1 < len(xs) else xs[i] for i in range(0, len(xs), 2)]
    return xs[0]


def make_kernel(S, D, H, F, *, TQ=256, CK=128, U=4, NA=2, SK=3, TP=512, TM=512, FC=512):
    Dh = D // H
    NQ = S // TQ
    NC = S // CK
    NSTEP = NQ * H
    qscale = (Dh ** -0.5) * math.log2(math.e)

    def kernel(x_h, wq_h, wkt_h, wvt_h, wo_h, wg_h, wu_h, wd_h, gw_h, out_h,
               x_v, wq_v, wkv_v, gw_v, wo_v, wg_v, wu_v, wd_v,
               qt_v, k_v, vt_v, grow_v, gcol_v, s_v, ot_v, h_v, out_v,
               sem_x, sem_w, sem_o):
        NP = S // TP
        x_cp = [pltpu.make_async_copy(x_h.at[pl.ds(i * TP, TP)], x_v.at[pl.ds(i * TP, TP)], sem_x.at[i])
                for i in range(NP)]
        wk_cp = pltpu.make_async_copy(wkt_h, wkv_v.at[pl.ds(0, Dh)], sem_w.at[0])
        wv_cp = pltpu.make_async_copy(wvt_h, wkv_v.at[pl.ds(Dh, Dh)], sem_w.at[1])
        gw_cp = pltpu.make_async_copy(gw_h, gw_v, sem_w.at[2])
        wq_cp = pltpu.make_async_copy(wq_h, wq_v, sem_w.at[3])
        wo_cp = pltpu.make_async_copy(wo_h, wo_v, sem_w.at[4])
        wg_cp = pltpu.make_async_copy(wg_h, wg_v, sem_w.at[5])
        wu_cp = pltpu.make_async_copy(wu_h, wu_v, sem_w.at[6])
        wd_cp = pltpu.make_async_copy(wd_h, wd_v, sem_w.at[7])

        wk_cp.start(); wv_cp.start(); gw_cp.start()
        x_cp[0].start(); wq_cp.start()
        for i in range(1, NP):
            x_cp[i].start()
        wg_cp.start(); wu_cp.start(); wd_cp.start(); wo_cp.start()

        wk_cp.wait(); wv_cp.wait(); gw_cp.wait()
        gw = gw_v[...].astype(F32)
        gw_row = jnp.concatenate([gw[r:r + 1, :] for r in range(D // 128)], axis=1)
        wkv_v[pl.ds(2 * Dh, 16), :] = jnp.broadcast_to(gw_row, (16, D)).astype(BF)
        for i in range(NP):
            x_cp[i].wait()
            xb = x_v[pl.ds(i * TP, TP), :]
            kvg = lax.dot_general(wkv_v[...], xb, NT, preferred_element_type=F32)
            g = jax.nn.sigmoid(kvg[2 * Dh:2 * Dh + 8])
            vt_v[:, pl.ds(i * TP, TP)] = _u32(kvg[Dh:2 * Dh].astype(BF))
            for t in range(TP // TQ):
                grow_v[i * (TP // TQ) + t] = g[:, t * TQ:(t + 1) * TQ]
            kg = jnp.concatenate([kvg[:Dh], jnp.broadcast_to(1.0 - g[:1], (128 - Dh, TP))], axis=0).T
            k_v[pl.ds(i * TP // 2, TP // 2), :] = _u32(kg[:, :Dh].astype(BF))
            gcol_v[pl.ds(i * TP, TP), :] = jnp.broadcast_to(kg[:, 127:128], (TP, 128))
            if i == 0:
                wq_cp.wait()
            q = jnp.dot(xb, wq_v[...], preferred_element_type=F32) * qscale
            for t in range(TP // TQ):
                qt = _u32(q[t * TQ:(t + 1) * TQ].T.astype(BF))
                qt_v[pl.ds((i * (TP // TQ) + t) * H, H)] = qt.reshape(H, Dh // 2, TQ)

        def qk(n, slot, c, m8):
            qh = _bf(qt_v[n])
            s = jnp.dot(_bf(k_v[pl.ds(c * CK // 2, CK // 2), :]), qh, preferred_element_type=F32)
            s_v[slot, pl.ds(c * CK, CK), :] = s
            for i in range(CK // 8):
                a = i % NA
                t = s[i * 8:(i + 1) * 8]
                m8[a] = t if m8[a] is None else jnp.maximum(m8[a], t)

        def fin_max(m8):
            m = jnp.max(_tree(jnp.maximum, m8), axis=0, keepdims=True)
            for a in range(NA):
                m8[a] = None
            return m

        m8 = [None] * NA
        for c in range(NC):
            qk(0, 0, c, m8)
        m0 = fin_max(m8)
        for c in range(SK):
            qk(1, 1, c, m8)

        def attn_body(it, carry):
            m_cur, m8 = carry
            m8 = list(m8)
            n0 = it * U
            grow = grow_v[n0 // H]
            for j in range(U):
                n = n0 + j
                cur = j % 2
                mb = jnp.broadcast_to(m_cur, (8, TQ))
                l8 = [None] * NA
                o = None
                m_next = None
                for c in range(NC):
                    cq = c + SK
                    if cq < NC:
                        qk(jnp.minimum(n + 1, NSTEP - 1), 1 - cur, cq, m8)
                        if cq == NC - 1:
                            m_next = fin_max(m8)
                    else:
                        qk(jnp.minimum(n + 2, NSTEP - 1), cur, cq - NC, m8)
                    sp = s_v[cur, pl.ds(c * CK, CK), :]
                    p = jnp.exp2(sp.reshape(CK // 8, 8, TQ) - mb[None])
                    for i in range(CK // 8):
                        a = i % NA
                        l8[a] = p[i] if l8[a] is None else l8[a] + p[i]
                    oc = jnp.dot(_bf(vt_v[:, pl.ds(c * CK, CK)]), p.reshape(CK, TQ).astype(BF),
                                 preferred_element_type=F32)
                    o = oc if o is None else o + oc
                l = jnp.sum(_tree(jnp.add, l8), axis=0, keepdims=True)
                ot_v[n] = _u32((o * (grow[:1] / l)).astype(BF))
                m_cur = m_next
            return m_cur, tuple(m8)

        lax.fori_loop(0, NSTEP // U, attn_body, (m0, tuple(m8)))

        wg_cp.wait(); wu_cp.wait(); wd_cp.wait(); wo_cp.wait()

        def out_cp(i):
            r = pl.ds(pl.multiple_of(i * TM, TM), TM)
            return pltpu.make_async_copy(out_v.at[r], out_h.at[r], sem_o.at[i])

        def ffn_body(i, _):
            r0 = pl.multiple_of(i * TM, TM)
            xb = x_v[pl.ds(r0, TM), :]
            for c in range(F // FC):
                gate = jnp.dot(xb, wg_v[:, pl.ds(c * FC, FC)], preferred_element_type=F32)
                up = jnp.dot(xb, wu_v[:, pl.ds(c * FC, FC)], preferred_element_type=F32)
                h_v[:, pl.ds(c * FC, FC)] = _u32((jnp.maximum(gate, 0.0) * up).astype(BF))
            ob = jnp.concatenate(
                [_bf(ot_v[pl.ds((i * (TM // TQ) + t) * H, H)].reshape(D // 2, TQ)).T for t in range(TM // TQ)], axis=0)
            a = jnp.dot(ob, wo_v[...], preferred_element_type=F32)
            b = jnp.dot(_bf(h_v[...]), wd_v[...], preferred_element_type=F32)
            gc = gcol_v[pl.ds(r0, TM), :]
            out = a + b * jnp.concatenate([gc] * (D // 128), axis=1)
            out_v[pl.ds(r0, TM), :] = out.astype(BF)
            out_cp(i).start()
            return 0

        lax.fori_loop(0, S // TM, ffn_body, 0)
        for i in range(S // TM):
            out_cp(i).wait()

    scratch = [
        pltpu.VMEM((S, D), BF), pltpu.VMEM((D, D), BF), pltpu.VMEM((2 * Dh + 16, D), BF), pltpu.VMEM((D // 128, 128), BF),
        pltpu.VMEM((D, D), BF), pltpu.VMEM((D, F), BF), pltpu.VMEM((D, F), BF), pltpu.VMEM((F, D), BF),
        pltpu.VMEM((NSTEP, Dh // 2, TQ), U32), pltpu.VMEM((S // 2, Dh), U32), pltpu.VMEM((Dh // 2, S), U32),
        pltpu.VMEM((NQ, 8, TQ), F32), pltpu.VMEM((S, 128), F32), pltpu.VMEM((2, S, TQ), F32),
        pltpu.VMEM((NSTEP, Dh // 2, TQ), U32), pltpu.VMEM((TM // 2, F), U32), pltpu.VMEM((S, D), BF),
        pltpu.SemaphoreType.DMA((S // TP,)), pltpu.SemaphoreType.DMA((8,)), pltpu.SemaphoreType.DMA((S // TM,)),
    ]
    return kernel, scratch


def build(**kw):
    def fn(A_x, A_wq, A_wk, A_wv, A_wo, B_x, B_W_gate, B_W_up, B_W_down, gate_w):
        del B_x
        B, S, D = A_x.shape
        H = 32
        F = B_W_gate.shape[1]
        kernel, scratch = make_kernel(S, D, H, F, **kw)
        out = pl.pallas_call(
            kernel,
            out_shape=jax.ShapeDtypeStruct((S, D), A_x.dtype),
            in_specs=[pl.BlockSpec(memory_space=pl.ANY)] * 9,
            out_specs=pl.BlockSpec(memory_space=pl.ANY),
            scratch_shapes=scratch,
            compiler_params=pltpu.CompilerParams(vmem_limit_bytes=110 * 2 ** 20),
            name="fused",
        )(A_x.reshape(S, D), A_wq, A_wk.T, A_wv.T, A_wo, B_W_gate, B_W_up, B_W_down, gate_w.reshape(D // 128, 128))
        return out.reshape(B, S, D)
    return fn


@jax.jit
def pallas_gated_mix__grouped_kv_mqa__glu_gated_reglu__prompt_kernel(
    A_x: jax.Array,
    A_wq: jax.Array,
    A_wk: jax.Array,
    A_wv: jax.Array,
    A_wo: jax.Array,
    B_x: jax.Array,
    B_W_gate: jax.Array,
    B_W_up: jax.Array,
    B_W_down: jax.Array,
    gate_w: jax.Array,
):
    return build()(A_x, A_wq, A_wk, A_wv, A_wo, B_x, B_W_gate, B_W_up, B_W_down, gate_w)
```

```python
import contextlib
import functools
import math

import jax
import jax.numpy as jnp
from jax import lax
from jax.experimental import pallas as pl
from jax.experimental.pallas import tpu as pltpu

BF = jnp.bfloat16
F32 = jnp.float32
U32 = jnp.uint32
NT = (((1,), (1,)), ((), ()))


def _bf(x):
    return pltpu.bitcast(x, BF)


def _dot(a, b):
    return jnp.dot(a, b, preferred_element_type=F32)


def _ds(start, size, align):
    return pl.ds(start if isinstance(start, int) else pl.multiple_of(start, align), size)


def _run(jobs):
    for job in jobs:
        job()


def _part(jobs, k, n):
    return jobs[k * len(jobs) // n:(k + 1) * len(jobs) // n] if k < n else []


_LHS = ((0, 1, 3), (2, 1, 3), (0,), (3,), (0, 1, 1), (2, -1, 0), (1, -1, 3))
_RHS = ((0, 1, 3), (0,), (1, -1, 3), (2, -1, 0), (3,), (0, 1, 1), (2, 1, 3))


def _operand(rule, block):
    if len(rule) == 1:
        return block(rule[0])
    a, b = block(rule[0]), block(rule[2])
    return a + b if rule[1] > 0 else a - b


def _form_jobs(rules, depth, get, put, rows):
    def job(r, p1):
        if depth == 1:
            block = [get(q // 2, q % 2, r).astype(F32) for q in range(4)]
        else:
            block = [_operand(rules[p1], lambda q1: get(2 * (q1 // 2) + q // 2, 2 * (q1 % 2) + q % 2, r).astype(F32))
                     for q in range(4)]
        for p2 in range(7):
            put(7 * p1 + p2, r, _operand(rules[p2], block.__getitem__).astype(BF))
    return [functools.partial(job, r, p1) for r in range(0, rows, 16) for p1 in range(7 ** (depth - 1))]


_ORDER = (1, 3, 0, 2, 4, 5, 6)


def _combine(product, save, load, emit):
    def take(j, key, v):
        if j < 5:
            save(j, key, v)
        if j == 3:
            emit(2, key, load(1, key) + v)
        elif j == 4:
            emit(1, key, load(2, key) + v)
        elif j == 5:
            emit(3, key, (load(0, key) - load(1, key)) + (load(2, key) + v))
        elif j == 6:
            emit(0, key, (load(0, key) + load(3, key)) + (v - load(4, key)))
    for j in _ORDER:
        product(j, functools.partial(take, j))


def _strassen2(product, rows, width, m_ref, zero, emit, side, before=None, extra=None):
    count = [0]

    def piece(n, r, width):
        return m_ref.at[zero + n, pl.ds(r % 128, 16), pl.ds((r // 128) * width, width)]

    def outer(j1, take1):
        base = 20 + 5 * (j1 % 2)

        def save(j, r, v):
            piece(base + j, r, width)[...] = v

        def inner(j2, take2):
            res = product(7 * j1 + j2)
            for r in range(0, rows, 16):
                take2(r, res[r:r + 16])
            side(count[0])
            count[0] += 1

        if before is not None:
            before(j1)
        _combine(inner, save, lambda j, r: piece(base + j, r, width)[...],
                 lambda q, r, v: take1((q, r), v if extra is None else v + extra(j1, q, r)))

    def save(j, key, v):
        piece(4 * j + key[0], key[1], width)[...] = v

    _combine(outer, save, lambda j, key: piece(4 * j + key[0], key[1], width)[...],
             lambda q1, key, v: emit(2 * (q1 // 2) + key[0] // 2, 2 * (q1 % 2) + key[0] % 2, key[1], v))


def make_kernel(S, D, H, F, *, PH=15, H0=2, O0=28, TW=2, OU=0, FL=0, ZU=0, KV=0, GP=5, U=16, SK=3, HP=21, WP=49, SC=0):
    Dh = D // H
    TQ = 256
    CK = 128
    NC = S // CK
    NSTEP = (S // TQ) * H
    TM = 2 * TQ
    NB = S // TM
    R = TM // 4
    DK = D // 4
    FC = 512
    NF = F // FC
    HD = D // 2
    qscale = (Dh ** -0.5) * math.log2(math.e)
    scope = jax.named_scope if SC else (lambda name: contextlib.nullcontext())

    def kernel(x_h, wq_h, wkt_h, wvt_h, wo_h, wg_h, wu_h, wd_h, gw_h, out_h,
               a_v, w_v, m_v, k_v, vt_v, g_v, ot_v, raw_v, rawd_v, zero_s, sem):
        @pl.loop(0, 3, unroll=False)
        def _(i):
            zero_s[0] = 2 - i

        def half_cp(w_h, c, slot, half):
            return pltpu.make_async_copy(w_h.at[:, _ds(c * FC, FC, FC)], raw_v.at[slot, half], sem.at[2 * slot + half])

        def up_cp(c, slot):
            return [half_cp(wg_h, c, slot, 0), half_cp(wu_h, c, slot, 1)]

        def down_cp(c, slot):
            return pltpu.make_async_copy(wd_h.at[_ds(c * FC, FC, FC)], rawd_v.at[slot], sem.at[NB + 7 + slot])

        def up_jobs(slot, r0, rows, zero):
            jobs = []
            for half in range(2):
                def put(p, r, v, half=half):
                    w_v.at[p, _ds(slot * 128 + r0 // 2, rows // 2, 8)].bitcast(BF)[pl.ds(r, 16), _ds((zero + half) * 128, 128, 128)] = v
                jobs += _form_jobs(_RHS, 2, lambda a, b, r, half=half:
                                   raw_v[slot, half, _ds(r0 + a * DK + r, 16, 16), pl.ds(b * 128, 128)], put, rows)
            return jobs

        def g_rows(row, n):
            return g_v[_ds(row, n, 8), :]

        def attention(qt_v, gt_v, wo_v):
            wo_cp = pltpu.make_async_copy(wo_h, wo_v, sem.at[4])

            def project(x_v, wkv_v, gw_v, wt_v):
                zero = zero_s[0]
                x_cp = [pltpu.make_async_copy(x_h.at[pl.ds(i * TM, TM)], x_v.at[pl.ds(i * TM, TM)], sem.at[4 + i])
                        for i in range(NB)]
                small = [pltpu.make_async_copy(wkt_h, wkv_v.at[pl.ds(0, Dh)], sem.at[4 + NB]),
                         pltpu.make_async_copy(wvt_h, wkv_v.at[pl.ds(Dh, Dh)], sem.at[5 + NB]),
                         pltpu.make_async_copy(gw_h, gw_v, sem.at[6 + NB])]
                quarters = ((0, 0), (1, 0), (1, 1), (0, 1))
                wq_cp = [pltpu.make_async_copy(wq_h.at[pl.ds(a * HD, HD), pl.ds(b * HD, HD)],
                                               raw_v.at[1, b, pl.ds(a * HD, HD)], sem.at[2 * a + b])
                         for a, b in quarters]

                def kvg(i):
                    t = lax.dot_general(wkv_v[...], x_v[_ds(i * TM, TM, TM), :], NT, preferred_element_type=F32)
                    g = jax.nn.sigmoid(t[2 * Dh:2 * Dh + 1])
                    vt_v.bitcast(BF)[:, _ds(i * TM, TM, TM)] = t[Dh:2 * Dh].astype(BF)
                    kg = jnp.concatenate([t[:Dh], jnp.broadcast_to(g, (128 - Dh, TM))], axis=0).T
                    k_v[_ds(i * (TM // 2), TM // 2, TM // 2), :] = pltpu.bitcast(kg[:, :Dh].astype(BF), U32)
                    g_v[_ds(i * TM, TM, TM), :] = jnp.broadcast_to(1.0 - kg[:, 127:128], (TM, 128))
                    for a1 in range(2):
                        gt_v[2 * i + a1] = g[:, a1 * TQ:(a1 + 1) * TQ]

                def x_jobs(i):
                    def put(p, r, v):
                        a_v.at[i, p].bitcast(BF)[pl.ds(r, 16), _ds(zero * 128, DK, 128)] = v
                    return _form_jobs(_LHS, 2, lambda a, b, r: x_v[_ds(i * TM + a * R + r, 16, 16), pl.ds(b * DK, DK)], put, R)

                def wq_jobs():
                    def put(p, r, v):
                        w_v.at[p, pl.ds(128, 128)].bitcast(BF)[pl.ds(r, 16), _ds(zero * 128, DK, 128)] = v
                    return _form_jobs(_RHS, 2, lambda a, b, r:
                                      _bf(wt_v[pl.ds((b * DK + r) // 2, 8), pl.ds(a * DK, DK)]), put, DK)

                def wq_transposes(n):
                    def job(r, c):
                        a, b = quarters[n]
                        wt_v.bitcast(BF)[pl.ds(b * HD + c, 128), _ds(a * HD + r + zero * 128, 128, 128)] = (
                            raw_v[1, b, pl.ds(a * HD + r, 128), pl.ds(c, 128)].T)
                    return [functools.partial(job, r, c) for c in range(0, HD, 128) for r in range(0, HD, 128)]

                def q_block(i, side):
                    groups = [x_jobs(i)[j::7] for j in _ORDER[1:]] + [x_jobs(jnp.minimum(i + 1, NB - 1))[_ORDER[0]::7]]

                    def emit(a, b, r, v):
                        dst = qt_v.at[(2 * i + a // 2) * H + (b * DK + r) // Dh].bitcast(BF)
                        dst[pl.ds(r % Dh, 16), pl.ds((a % 2) * R, R)] = (v * qscale).astype(BF)

                    def product(p):
                        return lax.dot_general(_bf(w_v[p, pl.ds(128, 128), :]), _bf(a_v[i, p, :, :DK]), NT,
                                               preferred_element_type=F32)

                    _strassen2(product, DK, R, m_v, zero, emit,
                               lambda k: (_run(_part(groups[k // 7], k % 7, GP)), side(k)))

                w_groups = [wq_jobs()[j::7] for j in _ORDER]
                _run([cp.start for cp in [wq_cp[0]] + small + [x_cp[0], wq_cp[1]]])
                wq_cp[0].wait()
                _run(wq_transposes(0) + w_groups[0])
                _run([cp.wait for cp in small])
                gw = gw_v[...].astype(F32)
                gw_row = jnp.concatenate([gw[r:r + 1, :] for r in range(D // 128)], axis=1)
                wkv_v[pl.ds(2 * Dh, 16), :] = jnp.broadcast_to(gw_row, (16, D)).astype(BF)
                _run([cp.start for cp in wq_cp[2:]])
                x_cp[0].wait()
                wq_cp[1].wait()
                _run(x_jobs(0)[_ORDER[0]::7])
                kvg(0)
                _run(wq_transposes(1))

                def first(k):
                    n, k2 = divmod(k, 7)
                    if k == TW:
                        _run([cp.start for cp in x_cp[1:]])
                        _run([cp.wait for cp in wq_cp[2:]])
                    if n == 0 and k > TW:
                        _run(_part(wq_transposes(2), k - TW - 1, 6 - TW))
                    if n == 1:
                        _run(_part(wq_transposes(3), k2, 6))
                    if n < 6:
                        _run(_part(w_groups[n + 1], k2, GP))
                    if k == 41:
                        _run([cp.start for cp in up_cp(0, 0) + up_cp(1, 1) + [wo_cp, down_cp(0, 0)]])
                        _run([cp.wait for cp in x_cp[1:]])

                q_block(0, first)

                def body(i, _):
                    q_block(i, lambda k: kvg(i) if k == KV else None)
                    return 0

                lax.fori_loop(1, NB, body, 0)

            with scope("proj"):
                if PH & 1: pl.run_scoped(project, pltpu.VMEM((S, D), BF), pltpu.VMEM((2 * Dh + 16, D), BF),
                              pltpu.VMEM((D // 128, 128), BF), pltpu.VMEM((D // 2, D), U32))
            _run([cp.wait for cp in up_cp(0, 0) + [wo_cp]])

            def attend(s_v, o_v):
                def scores(n, slot, c, m8):
                    s = _dot(_bf(k_v[pl.ds(c * CK // 2, CK // 2), :]), _bf(qt_v[n]))
                    s_v[slot, pl.ds(c * CK, CK), :] = s
                    for i in range(CK // 8):
                        t = s[i * 8:(i + 1) * 8]
                        m8[i % 2] = t if m8[i % 2] is None else jnp.maximum(m8[i % 2], t)

                def row_max(m8):
                    m = jnp.max(jnp.maximum(m8[0], m8[1]), axis=0, keepdims=True)
                    m8[0] = m8[1] = None
                    return m

                def body(it, carry):
                    m_cur, m8 = carry
                    m8 = list(m8)
                    g = gt_v[it * U // H]
                    jobs = up_jobs(0, it * (DK * U // NSTEP), DK * U // NSTEP, 0)
                    rows = HD * U // NSTEP
                    for half in range(2):
                        def put(p, r, v, half=half):
                            w_v.at[49 + p, _ds(half * 256 + it * (rows // 2), rows // 2, 8)].bitcast(BF)[pl.ds(r, 16), :] = v
                        jobs += _form_jobs(_RHS, 1, lambda a, b, r, half=half:
                                           wo_v[_ds(it * rows + a * HD + r, 16, 16), pl.ds(b * HD + half * DK, DK)], put, rows)
                    for j in range(U):
                        n = it * U + j
                        cur = j % 2
                        mb = jnp.broadcast_to(m_cur, (8, TQ))
                        l8 = [None, None]
                        for c in range(NC):
                            cq = c + SK
                            if cq < NC:
                                scores(jnp.minimum(n + 1, NSTEP - 1), 1 - cur, cq, m8)
                                if cq == NC - 1:
                                    m_cur = row_max(m8)
                            else:
                                scores(jnp.minimum(n + 2, NSTEP - 1), cur, cq - NC, m8)
                            p = jnp.exp2(s_v[cur, pl.ds(c * CK, CK), :].reshape(CK // 8, 8, TQ) - mb[None])
                            for i in range(CK // 8):
                                l8[i % 2] = p[i] if l8[i % 2] is None else l8[i % 2] + p[i]
                            o = _dot(_bf(vt_v[:, pl.ds(c * CK, CK)]), p.reshape(CK, TQ).astype(BF))
                            if c > 0:
                                o = o_v[...] + o
                            if c < NC - 1:
                                o_v[...] = o
                        _run(_part(jobs, j, U))
                        l = jnp.sum(l8[0] + l8[1], axis=0, keepdims=True)
                        ot_v.at[n].bitcast(BF)[...] = (o * (g / l)).astype(BF)
                    return m_cur, tuple(m8)

                m8 = [None, None]
                for c in range(NC):
                    scores(0, 0, c, m8)
                m0 = row_max(m8)
                for c in range(SK):
                    scores(1, 1, c, m8)
                lax.fori_loop(0, NSTEP // U, body, (m0, tuple(m8)))

            with scope("attn"):
                if PH & 2: pl.run_scoped(attend, pltpu.VMEM((2, S, TQ), F32), pltpu.VMEM((Dh, TQ), F32))

        pl.run_scoped(attention, pltpu.VMEM((NSTEP, Dh // 2, TQ), U32), pltpu.VMEM((S // TQ, 1, TQ), F32),
                      pltpu.VMEM((D, D), BF))

        def ffn(h0_v, h1_v, oa_v, y_v, out_v):
            h_v = (h0_v, h1_v)

            def down_jobs(c, slot, r0, rows):
                jobs = []
                for half in range(2):
                    def put(p, r, v, half=half):
                        w_v.at[p, _ds(256 + c * 64 + r0 // 2, rows // 2, 8)].bitcast(BF)[pl.ds(r, 16), pl.ds(half * 128, 128)] = v
                    jobs += _form_jobs(_RHS, 2, lambda a, b, r, half=half:
                                       rawd_v[slot, _ds(r0 + a * 128 + r, 16, 16), pl.ds(b * DK + half * 128, 128)], put, rows)
                return jobs

            def act_jobs(n, src, zero):
                def put(p, r, v):
                    a_v.at[n % NB, p].bitcast(BF)[pl.ds(r, 16), _ds(DK + (n // NB) * 128, 128, 128)] = v
                return _form_jobs(_LHS, 2, lambda a, b, r: src[zero, 4 * a + b, pl.ds(r, 16), :], put, R)

            def o_jobs(i, slot, a2, c):
                def block(q):
                    n = (2 * i + q // 2) * H + (q % 2) * (H // 2) + c * (128 // Dh)
                    return _bf(ot_v[pl.ds(n, 128 // Dh), :, _ds(a2 * R, R, R)].reshape(64, R)).astype(F32)

                def job(p):
                    oa_v.at[slot, p, a2].bitcast(BF)[:, _ds(c * 128, 128, 128)] = _operand(_LHS[p], block).T.astype(BF)
                return [functools.partial(job, p) for p in range(7)]

            def body(t, _):
                c, half = t // 2, t % 2
                slot = c % 2
                zero = zero_s[0]

                @pl.when(half == 0)
                def _():
                    @pl.when(c + 1 < NF)
                    def _():
                        _run([cp.wait for cp in up_cp(c + 1, 1 - slot)])
                        down_cp(c + 1, 1 - slot).start()

                    @pl.when(c + 2 < NF)
                    def _():
                        _run([cp.start for cp in up_cp(c + 2, slot)])

                    down_cp(c, slot).wait()

                weights = [up_jobs(1 - slot, half * (DK // 2), DK // 2, zero if ZU else 0), down_jobs(c, slot, half * 64, 64)]
                weights = [_part(weights[0], 0, 4) + _part(weights[0], 1, 4) + _part(weights[0], 2, 4),
                           _part(weights[0], 3, 4) + weights[1]]
                first = o_jobs(0, 0, half, c % (HD // 128))
                for u in range(2):
                    i = 2 * half + u
                    prev = act_jobs(jnp.maximum(2 * t + u - 1, 0), h_v[1 - u], zero)

                    def emit(a, b, r, v):
                        h_v[u][0, 4 * a + b, pl.ds(r, 16), :] = (
                            jnp.maximum(v[:, :128], 0.0) * v[:, 128:] * g_rows(i * TM + a * R + r, 16))

                    _strassen2(lambda p: _dot(_bf(a_v[i, p, :, :DK]), _bf(w_v[p, _ds(slot * 128, 128, 128), :])),
                               R, 256, m_v, zero, emit, lambda k: _run((_part(first, k - O0, 14) if u == OU and k >= O0 else []) + _part(weights[u], k, WP) + (_part(prev, k - H0, HP - H0) if k >= H0 else [])))
                return 0

            with scope("up"):
                h1_v[...] = jnp.zeros(h1_v.shape, F32)
                if PH & 4: lax.fori_loop(0, 2 * NF, body, 0)

            def out_cp(t, q):
                return [pltpu.make_async_copy(
                    out_v.at[t, b, pl.ds((q // 2) * TQ, TQ)],
                    out_h.at[_ds((t // 2) * TM + (q // 2) * TQ, TQ, TQ), _ds(b * DK + (t % 2) * 128, 128, 128)],
                    sem.at[NB + 9]) for b in (2 * (q % 2), 2 * (q % 2) + 1)]

            def body(t, _):
                i, half = t // 2, t % 2
                zero = zero_s[0]
                cols = _ds(half * 128, 128, 128)

                jobs = [job for c in range(HD // 128) for job in o_jobs(jnp.minimum(i + 1, NB - 1), 1 - i % 2, half, c)]

                def attn_product(j):
                    wo = jnp.concatenate([_bf(w_v[49 + j, pl.ds(h * 256, 256), cols]) for h in range(2)], axis=1)
                    y_v[j % 2] = _dot(_bf(oa_v[i % 2, j].reshape(R, HD)), wo)

                def side(k):
                    _run(_part(jobs, k, 42))
                    if k == 42:
                        _run([cp.start for q in (2, 1, 3) for cp in out_cp(t, q)])

                def emit(a, b, r, v):
                    out_v[t, b, pl.ds(a * R + r, 16), :] = v.astype(BF)

                _strassen2(lambda p: _dot(_bf(a_v[i, p, :, DK:]), _bf(w_v[p, pl.ds(256, NF * 64), cols])),
                           R, 128, m_v, zero, emit, side, attn_product,
                           lambda j, q, r: y_v[zero + j % 2, pl.ds((q // 2) * R + r, 16), pl.ds((q % 2) * 128, 128)])
                _run([cp.start for cp in out_cp(t, 0)])
                return 0

            with scope("down"):
                _run(act_jobs(NB * NF - 1, h1_v, 0))
                if PH & 8: lax.fori_loop(0, 2 * NB, body, 0)
                pltpu.make_async_copy(out_v, out_v, sem.at[NB + 9]).wait()

        pl.run_scoped(ffn, pltpu.VMEM((1, 16, R, 128), F32), pltpu.VMEM((1, 16, R, 128), F32),
                      pltpu.VMEM((2, 7, 2, R // 2, HD), U32), pltpu.VMEM((2, 2 * R, 256), F32), pltpu.VMEM((2 * NB, 4, TM, 128), BF))

    scratch = [
        pltpu.VMEM((NB, 49, R // 2, DK + NF * 128), U32),
        pltpu.VMEM((49 + 7, 256 + NF * 64, 256), U32),
        pltpu.VMEM((30, R, 256), F32),
        pltpu.VMEM((S // 2, Dh), U32),
        pltpu.VMEM((Dh // 2, S), U32),
        pltpu.VMEM((S, 128), F32),
        pltpu.VMEM((NSTEP, Dh // 2, TQ), U32),
        pltpu.VMEM((2, 2, D, FC), BF),
        pltpu.VMEM((2, FC, D), BF),
        pltpu.SMEM((1,), jnp.int32),
        pltpu.SemaphoreType.DMA((NB + 10,)),
    ]
    return kernel, scratch


def build(**kw):
    def fn(A_x, A_wq, A_wk, A_wv, A_wo, B_x, B_W_gate, B_W_up, B_W_down, gate_w):
        del B_x
        B, S, D = A_x.shape
        kernel, scratch = make_kernel(S, D, 32, B_W_gate.shape[1], **kw)
        out = pl.pallas_call(
            kernel,
            out_shape=jax.ShapeDtypeStruct((S, D), A_x.dtype),
            in_specs=[pl.BlockSpec(memory_space=pl.ANY)] * 9,
            out_specs=pl.BlockSpec(memory_space=pl.ANY),
            scratch_shapes=scratch,
            compiler_params=pltpu.CompilerParams(vmem_limit_bytes=127 * 2 ** 20, disable_bounds_checks=True,
                flags={0: None, 1: {'XLA_TPU_FORCE_LP_LLO_SCHEDULER': True}, 2: {'XLA_TPU_EVENLY_DISTRIBUTE_CRITICAL_NODES': True}}[kw.get('FL', 0)]),
            name="fused",
        )(A_x.reshape(S, D), A_wq, A_wk.T, A_wv.T, A_wo, B_W_gate, B_W_up, B_W_down, gate_w.reshape(D // 128, 128))
        return out.reshape(B, S, D)
    return fn


@jax.jit
def pallas_gated_mix__grouped_kv_mqa__glu_gated_reglu__prompt_kernel(
    A_x: jax.Array,
    A_wq: jax.Array,
    A_wk: jax.Array,
    A_wv: jax.Array,
    A_wo: jax.Array,
    B_x: jax.Array,
    B_W_gate: jax.Array,
    B_W_up: jax.Array,
    B_W_down: jax.Array,
    gate_w: jax.Array,
):
    return build()(A_x, A_wq, A_wk, A_wv, A_wo, B_x, B_W_gate, B_W_up, B_W_down, gate_w)
```

```python
import functools
import math

import jax
import jax.numpy as jnp
from jax import lax
from jax.experimental import pallas as pl
from jax.experimental.pallas import tpu as pltpu

BF = jnp.bfloat16
F32 = jnp.float32
U32 = jnp.uint32
NT = (((1,), (1,)), ((), ()))


def _bf(x):
    return pltpu.bitcast(x, BF)


def _dot(a, b):
    return jnp.dot(a, b, preferred_element_type=F32)


def _ds(start, size, align):
    return pl.ds(start if isinstance(start, int) else pl.multiple_of(start, align), size)


def _run(jobs):
    for job in jobs:
        job()


def _part(jobs, k, first, end):
    if not first <= k < end:
        return []
    return jobs[(k - first) * len(jobs) // (end - first):(k + 1 - first) * len(jobs) // (end - first)]


_LHS = ((0, 1, 3), (2, 1, 3), (0,), (3,), (0, 1, 1), (2, -1, 0), (1, -1, 3))
_RHS = ((0, 1, 3), (0,), (1, -1, 3), (2, -1, 0), (3,), (0, 1, 1), (2, 1, 3))
_ORDER = (1, 3, 0, 2, 4, 5, 6)


def _operand(rule, block):
    if len(rule) == 1:
        return block(rule[0])
    a, b = block(rule[0]), block(rule[2])
    return a + b if rule[1] > 0 else a - b


def _operand_jobs(rules, get, put, rows):
    def job(r, p1):
        block = [_operand(rules[p1], lambda q1: get(2 * (q1 // 2) + q // 2, 2 * (q1 % 2) + q % 2, r).astype(F32))
                 for q in range(4)]
        for p2 in range(7):
            put(7 * p1 + p2, r, _operand(rules[p2], block.__getitem__).astype(BF))
    return [functools.partial(job, r, p1) for r in range(0, rows, 16) for p1 in range(7)]


def _combine(product, save, load, emit):
    def take(j, key, v):
        if j < 5:
            save(j, key, v)
        if j == 3:
            emit(2, key, load(1, key) + v)
        elif j == 4:
            emit(1, key, load(2, key) + v)
        elif j == 5:
            emit(3, key, (load(0, key) - load(1, key)) + (load(2, key) + v))
        elif j == 6:
            emit(0, key, (load(0, key) + load(3, key)) + (v - load(4, key)))
    for j in _ORDER:
        product(j, functools.partial(take, j))


def _strassen(product, shape, m_ref, zero, emit, side):
    rows, width = shape
    count = [0]

    def piece(n, r):
        return m_ref.at[zero + n, pl.ds(r % 128, 16), pl.ds((r // 128) * width, width)]

    def outer(j1, take1):
        base = 20 + 5 * (j1 % 2)

        def inner(j2, take2):
            res = product(7 * j1 + j2)
            for r in range(0, rows, 16):
                take2(r, res[r:r + 16])
            side(count[0])
            count[0] += 1

        def save(j, r, v):
            piece(base + j, r)[...] = v

        _combine(inner, save, lambda j, r: piece(base + j, r)[...], lambda q, r, v: take1((q, r), v))

    def save(j, key, v):
        piece(4 * j + key[0], key[1])[...] = v

    _combine(outer, save, lambda j, key: piece(4 * j + key[0], key[1])[...],
             lambda q1, key, v: emit(2 * (q1 // 2) + key[0] // 2, 2 * (q1 % 2) + key[0] % 2, key[1], v))


def _make_kernel(S, D, H, F):
    Dh = D // H
    TQ = 256
    CK = 128
    NC = S // CK
    NSTEP = (S // TQ) * H
    U = 16
    AHEAD = 4
    TM = 2 * TQ
    NB = S // TM
    R = TM // 4
    DK = D // 4
    HD = D // 2
    FC = 512
    NF = F // FC
    assert (D, Dh, NB, NF % 2, F) == (2 * FC, 32, 4, 1, NF * FC)
    qscale = (Dh ** -0.5) * math.log2(math.e)
    SEM_X, SEM_SMALL, SEM_DOWN, SEM_OUT = 4, 4 + NB, 7 + NB, 9 + NB

    def kernel(x_h, wq_h, wkt_h, wvt_h, wo_h, wg_h, wu_h, wd_h, gw_h, out_h,
               xa_v, ha_v, w_v, m_v, k_v, vt_v, g_v, ot_v, raw_v, rawd_v, zero_s, sem):
        @pl.loop(0, 3, unroll=False)
        def _(i):
            zero_s[0] = 2 - i

        def up_cp(c, slot):
            return [pltpu.make_async_copy(w_h.at[:, _ds(c * FC, FC, FC)], raw_v.at[slot, half], sem.at[2 * slot + half])
                    for half, w_h in enumerate((wg_h, wu_h))]

        def down_cp(c, slot):
            return pltpu.make_async_copy(wd_h.at[_ds(c * FC, FC, FC)], rawd_v.at[slot], sem.at[SEM_DOWN + slot])

        def up_jobs(slot, r0, rows):
            jobs = []
            for half in range(2):
                def put(p, r, v, half=half):
                    dst = w_v.at[p, _ds(slot * 128 + r0 // 2, rows // 2, 8)].bitcast(BF)
                    dst[pl.ds(r, 16), pl.ds(half * 128, 128)] = v
                jobs += _operand_jobs(_RHS, lambda a, b, r, half=half:
                                      raw_v[slot, half, _ds(r0 + a * DK + r, 16, 16), pl.ds(b * 128, 128)], put, rows)
            return jobs

        def wo_cp(slot, half):
            moves = ((0, 0, DK), (DK + 16, DK, HD - 16), (DK, DK + HD - 16, 16), (DK + HD, DK + HD, DK))
            return [pltpu.make_async_copy(wo_h.at[pl.ds(src, n), pl.ds(half * HD, HD)],
                                          raw_v.at[slot, half, pl.ds(dst, n)], sem.at[2 * slot + half])
                    for src, dst, n in moves]

        def o_row(unit):
            lo, hi = DK // 16, (DK + HD) // 16
            return jnp.where(unit == lo, hi - 1, jnp.where((unit > lo) & (unit < hi), unit - 1, unit))

        def anchor(i, p):
            return ha_v.at[i, 49], (p // 7) * 8, pl.ds((p % 7) * 128, 128)

        def project(qt_v, gt_v, x_v, wkv_v, gw_v):
            zero = zero_s[0]
            quarters = ((0, 0), (1, 0), (1, 1), (0, 1))
            wq_cp = [pltpu.make_async_copy(wq_h.at[pl.ds(a * HD, HD), pl.ds(b * HD, HD)],
                                           raw_v.at[1, b, pl.ds(a * HD, HD)], sem.at[2 * a + b]) for a, b in quarters]
            x0_cp = [pltpu.make_async_copy(x_h.at[pl.ds(a * TQ, TQ)], x_v.at[pl.ds(a * TQ, TQ)], sem.at[n])
                     for a, n in ((1, SEM_X), (0, SEM_OUT))]
            x_cp = [pltpu.make_async_copy(x_h.at[pl.ds(i * TM, TM)], x_v.at[pl.ds(i * TM, TM)], sem.at[SEM_X + i])
                    for i in range(1, NB)]
            small = [pltpu.make_async_copy(wkt_h, wkv_v.at[pl.ds(0, Dh)], sem.at[SEM_SMALL]),
                     pltpu.make_async_copy(wvt_h, wkv_v.at[pl.ds(Dh, Dh)], sem.at[SEM_SMALL + 1]),
                     pltpu.make_async_copy(gw_h, gw_v, sem.at[SEM_SMALL + 2])]

            def keys_values_gate(i):
                t = lax.dot_general(wkv_v[...], x_v[_ds(i * TM, TM, TM), :], NT, preferred_element_type=F32)
                g = jax.nn.sigmoid(t[2 * Dh:2 * Dh + 1])
                vt_v.bitcast(BF)[:, _ds(i * TM, TM, TM)] = t[Dh:2 * Dh].astype(BF)
                kg = jnp.concatenate([t[:Dh], jnp.broadcast_to(g, (128 - Dh, TM))], axis=0).T
                k_v[_ds(i * (TM // 2), TM // 2, TM // 2), :] = pltpu.bitcast(kg[:, :Dh].astype(BF), U32)
                g_v[_ds(i * TM, TM, TM), :] = jnp.broadcast_to(1.0 - kg[:, 127:128], (TM, 128))
                for a in range(2):
                    gt_v[2 * i + a] = g[:, a * TQ:(a + 1) * TQ]

            def x_jobs(i):
                def put(p, r, v):
                    cols = _ds(zero * 128, DK, 128) if isinstance(i, int) else pl.ds(0, DK)
                    xa_v.at[i, p].bitcast(BF)[pl.ds(r, 16), cols] = v
                    if r == 0:
                        ref, row, col = anchor(i, p)
                        ref.bitcast(BF)[pl.ds(2 * row, 16), col] = v[:, :128]
                return _operand_jobs(_LHS, lambda a, b, r: x_v[_ds(i * TM + a * R + r, 16, 16), pl.ds(b * DK, DK)], put, R)

            def wq_transposes(n):
                def job(r, c):
                    a, b = quarters[n]
                    dst = ot_v.at[zero + (b * HD + c) // DK].bitcast(BF)
                    dst[pl.ds((a * HD + r) // DK * DK + c % DK, 128), pl.ds(r % DK, 128)] = (
                        raw_v[1, b, pl.ds(a * HD + r, 128), pl.ds(c, 128)].T)
                return [functools.partial(job, r, c) for c in range(0, HD, 128) for r in range(0, HD, 128)]

            wq_jobs = []
            for c in range(0, DK, 128):
                def put_wq(p, r, v, c=c):
                    w_v.at[p, pl.ds(128, 128)].bitcast(BF)[pl.ds(r, 16), pl.ds(c, 128)] = v
                wq_jobs += _operand_jobs(_RHS, lambda a, b, r, c=c:
                                         _bf(ot_v[b, pl.ds((a * DK + r) // 2, 8), pl.ds(c, 128)]), put_wq, DK)

            def queries(i, side):
                after = i + 1 if isinstance(i, int) else jnp.minimum(i + 1, NB - 1)
                groups = [x_jobs(i)[j::7] for j in _ORDER[1:]] + [x_jobs(after)[_ORDER[0]::7]]

                def product(p):
                    w = w_v[p, pl.ds(128, 128), :]
                    if isinstance(i, int):
                        w = jnp.concatenate([w_v[p, pl.ds(128, 8), _ds(zero * 128, DK, 128)], w[8:]], axis=0)
                    return lax.dot_general(_bf(w), _bf(xa_v[i, p]), NT, preferred_element_type=F32)

                def emit(a, b, r, v):
                    dst = qt_v.at[(2 * i + a // 2) * H + (b * DK + r) // Dh].bitcast(BF)
                    dst[pl.ds(r % Dh, 16), pl.ds((a % 2) * R, R)] = (v * qscale).astype(BF)

                _strassen(product, (DK, R), m_v, zero, emit,
                          lambda k: (_run(_part(groups[k // 7], k % 7, 0, 7)), side(k)))

            _run([cp.start for cp in (wq_cp[0], x0_cp[0], wq_cp[1])])
            wq_cp[0].wait()
            _run([cp.start for cp in (wq_cp[2], x0_cp[1])])
            _run(wq_transposes(0) + wq_jobs[_ORDER[0]::7])
            x0_cp[0].wait()
            _run(x_jobs(0)[_ORDER[0]::7])
            _run([cp.start for cp in [wq_cp[3]] + small])
            wq_cp[1].wait()
            _run(wq_transposes(1))

            def first(k):
                if k == 3:
                    x_cp[0].start()
                    _run([cp.wait for cp in (wq_cp[2], x0_cp[1])])
                if k == 9:
                    _run([cp.start for cp in x_cp[1:]])
                    _run([cp.wait for cp in [wq_cp[3]] + small])
                    gw = gw_v[...].astype(F32)
                    gw_row = jnp.concatenate([gw[r:r + 1, :] for r in range(D // 128)], axis=1)
                    wkv_v[pl.ds(2 * Dh, 16), :] = jnp.broadcast_to(gw_row, (16, D)).astype(BF)
                if k == 14:
                    keys_values_gate(0)
                _run(_part(wq_transposes(2), k, 3, 7) + _part(wq_transposes(3), k, 9, 14))
                if k < 42:
                    _run(_part(wq_jobs[_ORDER[k // 7 + 1]::7], k % 7, 0, 7))
                if k == 41:
                    _run([cp.start for cp in up_cp(0, 0) + up_cp(1, 1) + [down_cp(0, 0)]])
                    _run([cp.wait for cp in x_cp])

            queries(0, first)

            @pl.loop(1, NB)
            def _(i):
                queries(i, lambda k: keys_values_gate(i) if k == 0 else None)

        def attend(qt_v, gt_v, s_v, o_v):
            def scores(n, slot, c, m8):
                s = _dot(_bf(k_v[pl.ds(c * CK // 2, CK // 2), :]), _bf(qt_v[n]))
                s_v[slot, pl.ds(c * CK, CK), :] = s
                for i in range(CK // 8):
                    t = s[i * 8:(i + 1) * 8]
                    m8[i % 2] = t if m8[i % 2] is None else jnp.maximum(m8[i % 2], t)

            def final_max(m8):
                m = jnp.max(jnp.maximum(m8[0], m8[1]), axis=0, keepdims=True)
                m8[0] = m8[1] = None
                return m

            def body(it, carry):
                m_max, m8 = carry
                m8 = list(m8)
                g = gt_v[it * U // H]
                jobs = up_jobs(0, it * (DK * U // NSTEP), DK * U // NSTEP)
                for j in range(U):
                    n = it * U + j
                    cur = j % 2
                    m = jnp.broadcast_to(m_max, (8, TQ))
                    l8 = [None, None]
                    for c in range(NC):
                        if c + AHEAD < NC:
                            scores(jnp.minimum(n + 1, NSTEP - 1), 1 - cur, c + AHEAD, m8)
                            if c + AHEAD == NC - 1:
                                m_max = final_max(m8)
                        else:
                            scores(jnp.minimum(n + 2, NSTEP - 1), cur, c + AHEAD - NC, m8)
                        p = jnp.exp2(s_v[cur, pl.ds(c * CK, CK), :].reshape(CK // 8, 8, TQ) - m[None])
                        for i in range(CK // 8):
                            l8[i % 2] = p[i] if l8[i % 2] is None else l8[i % 2] + p[i]
                        o = _dot(_bf(vt_v[:, pl.ds(c * CK, CK)]), p.reshape(CK, TQ).astype(BF))
                        if c > 0:
                            o = o_v[...] + o
                        if c < NC - 1:
                            o_v[...] = o
                    _run(_part(jobs, j, 0, U))
                    o = o * (g / jnp.sum(l8[0] + l8[1], axis=0, keepdims=True))
                    for part in range(2):
                        dst = ot_v.at[n // H, _ds(8 * o_row(2 * (n % H) + part), 8, 8)].bitcast(BF)
                        dst[...] = o[16 * part:16 * part + 16].astype(BF)
                return m_max, tuple(m8)

            m8 = [None, None]
            for c in range(NC):
                scores(0, 0, c, m8)
            m_max = final_max(m8)
            for c in range(AHEAD):
                scores(1, 1, c, m8)
            lax.fori_loop(0, NSTEP // U, body, (m_max, tuple(m8)))

        def attention(qt_v, gt_v):
            pl.run_scoped(functools.partial(project, qt_v, gt_v), pltpu.VMEM((S, D), BF),
                          pltpu.VMEM((2 * Dh + 16, D), BF), pltpu.VMEM((D // 128, 128), BF))
            _run([cp.wait for cp in up_cp(0, 0)])
            pl.run_scoped(functools.partial(attend, qt_v, gt_v), pltpu.VMEM((2, S, TQ), F32), pltpu.VMEM((Dh, TQ), F32))

        pl.run_scoped(attention, pltpu.VMEM((NSTEP, Dh // 2, TQ), U32), pltpu.VMEM((S // TQ, 1, TQ), F32))

        def ffn(h0_v, h1_v, on_v):
            h_v = (h0_v, h1_v)

            def down_jobs(c, slot, r0, rows):
                jobs = []
                for half in range(2):
                    def put(p, r, v, half=half):
                        dst = w_v.at[p, _ds(256 + c * 64 + r0 // 2, rows // 2, 8)].bitcast(BF)
                        dst[pl.ds(r, 16), pl.ds(half * 128, 128)] = v
                    jobs += _operand_jobs(_RHS, lambda a, b, r, half=half:
                                          rawd_v[slot, _ds(r0 + a * 128 + r, 16, 16), pl.ds(half * HD + b * 128, 128)],
                                          put, rows)
                return jobs

            def h_jobs(n, src, zero):
                def put(p, r, v):
                    ha_v.at[n % NB, p].bitcast(BF)[pl.ds(r, 16), _ds((n // NB) * 128, 128, 128)] = v
                return _operand_jobs(_LHS, lambda a, b, r: src[zero, 4 * a + b, pl.ds(r, 16), :], put, R)

            def o_jobs(i, r0, rows, zero):
                def put(p, r, v):
                    dst = ha_v.at[i, p, _ds(r0 // 2, rows // 2, 8)].bitcast(BF)
                    dst[pl.ds(r, 16), _ds((NF + zero) * 128, DK, 128)] = v
                return _operand_jobs(_LHS, lambda a, b, r:
                                     _bf(on_v[2 * i + a // 2, _ds(((a % 2) * R + r0 + r) // 2, 8, 8), pl.ds(b * DK, DK)]),
                                     put, rows)

            def o_transpose(tile, c):
                on_v.at[tile].bitcast(BF)[:, _ds(c * 128, 128, 128)] = _bf(ot_v[tile, _ds(c * 64, 64, 64), :]).T

            h1_v[...] = jnp.zeros(h1_v.shape, F32)

            @pl.loop(0, 2 * NF)
            def _(t):
                c, half = t // 2, t % 2
                slot = c % 2
                zero = zero_s[0]

                @pl.when(half == 0)
                def _():
                    _run([cp.wait for cp in up_cp(0, 1 - slot)])

                    @pl.when(c + 1 < NF)
                    def _():
                        down_cp(c + 1, 1 - slot).start()

                    @pl.when(c + 2 == NF)
                    def _():
                        _run([cp.start for n in range(2) for cp in wo_cp(slot, n)])

                    @pl.when(c + 2 < NF)
                    def _():
                        _run([cp.start for cp in up_cp(c + 2, slot)])

                    down_cp(c, slot).wait()

                weights = up_jobs(1 - slot, half * (DK // 2), DK // 2) + down_jobs(c, slot, half * 64, 64)
                early = [functools.partial(o_transpose, c % 4, 4 * half + n) for n in range(4)]
                early += o_jobs(0, (t % (R // 16)) * 16, 16, zero)
                for u in range(2):
                    i = 2 * half + u
                    before = h_jobs(jnp.maximum(2 * t + u - 1, 0), h_v[1 - u], zero)

                    def product(p):
                        ref, row, col = anchor(i, p)
                        x = [xa_v[i, p, pl.ds(r, 8), :] for r in range(0, R // 2, 8)]
                        x[0] = jnp.concatenate([ref[pl.ds(row, 8), col], xa_v[i, p, pl.ds(0, 8), 128:]], axis=1)
                        return _dot(_bf(jnp.concatenate(x, axis=0)), _bf(w_v[p, _ds(slot * 128, 128, 128), :]))

                    def emit(a, b, r, v):
                        h_v[u][0, 4 * a + b, pl.ds(r, 16), :] = (
                            jnp.maximum(v[:, :128], 0.0) * v[:, 128:] * g_v[_ds(i * TM + a * R + r, 16, 8), :])

                    _strassen(product, (R, 256), m_v, zero, emit,
                              lambda k: _run(_part(early, 49 * u + k, 77, 91) + _part(_part(weights, u, 0, 2), k, 0, 49)
                                             + _part(before, k, 2, 35)))

            _run(h_jobs(NB * NF - 1, h1_v, 0))

            @pl.loop(0, 2 * NB)
            def _(t):
                i, half = t // 2, t % 2
                cols = _ds(half * 128, 128, 128)
                jobs = o_jobs(jnp.minimum(i + 1, NB - 1), half * (R // 2), R // 2, 0)
                jobs += [functools.partial(o_transpose, jnp.minimum(t + 4, 2 * NB - 1), c) for c in range(D // 128)]

                def out_cp(q):
                    return pltpu.make_async_copy(
                        raw_v.at[i // 2, i % 2, _ds(half * TM + (q // 2) * TQ, TQ, TQ), pl.ds((q % 2) * DK, DK)],
                        out_h.at[_ds(i * TM + (q // 2) * TQ, TQ, TQ), _ds(half * HD + (q % 2) * DK, DK, DK)],
                        sem.at[SEM_OUT])

                def product(p):
                    w = jnp.concatenate([_bf(w_v[p, pl.ds(256, NF * 64), cols]), _bf(w_v[p, pl.ds(128, 128), cols])], axis=0)
                    return _dot(_bf(ha_v[i, p]), w)

                def emit(a, b, r, v):
                    raw_v[i // 2, i % 2, _ds(half * TM + a * R + r, 16, 16), pl.ds(b * 128, 128)] = v.astype(BF)

                def side(k):
                    _run(_part(jobs, k, 0, 42))
                    if k == 42:
                        _run([out_cp(q).start for q in (2, 1, 3)])

                _strassen(product, (R, 128), m_v, zero_s[0], emit, side)
                out_cp(0).start()

            pltpu.make_async_copy(raw_v, raw_v, sem.at[SEM_OUT]).wait()

        pl.run_scoped(ffn, pltpu.VMEM((1, 16, R, 128), F32), pltpu.VMEM((1, 16, R, 128), F32),
                      pltpu.VMEM((S // TQ, TQ // 2, D), U32))

    scratch = [
        pltpu.VMEM((NB, 49, R // 2, DK), U32),
        pltpu.VMEM((NB, 50, R // 2, NF * 128 + DK), U32),
        pltpu.VMEM((49, 256 + NF * 64, 256), U32),
        pltpu.VMEM((30, 128, 256), F32),
        pltpu.VMEM((S // 2, Dh), U32),
        pltpu.VMEM((Dh // 2, S), U32),
        pltpu.VMEM((S, 128), F32),
        pltpu.VMEM((S // TQ, D // 2, TQ), U32),
        pltpu.VMEM((2, 2, D, FC), BF),
        pltpu.VMEM((2, FC, D), BF),
        pltpu.SMEM((1,), jnp.int32),
        pltpu.SemaphoreType.DMA((SEM_OUT + 1,)),
    ]
    return kernel, scratch


@jax.jit
def pallas_gated_mix__grouped_kv_mqa__glu_gated_reglu__prompt_kernel(
    A_x: jax.Array,
    A_wq: jax.Array,
    A_wk: jax.Array,
    A_wv: jax.Array,
    A_wo: jax.Array,
    B_x: jax.Array,
    B_W_gate: jax.Array,
    B_W_up: jax.Array,
    B_W_down: jax.Array,
    gate_w: jax.Array,
):
    del B_x
    B, S, D = A_x.shape
    kernel, scratch = _make_kernel(S, D, D // A_wk.shape[1], B_W_gate.shape[1])
    out = pl.pallas_call(
        kernel,
        out_shape=jax.ShapeDtypeStruct((S, D), A_x.dtype),
        in_specs=[pl.BlockSpec(memory_space=pl.ANY)] * 9,
        out_specs=pl.BlockSpec(memory_space=pl.ANY),
        scratch_shapes=scratch,
        compiler_params=pltpu.CompilerParams(vmem_limit_bytes=127 * 2 ** 20, disable_bounds_checks=True),
        name="fused",
    )(A_x.reshape(S, D), A_wq, A_wk.T, A_wv.T, A_wo, B_W_gate, B_W_up, B_W_down, gate_w.reshape(D // 128, 128))
    return out.reshape(B, S, D)
```

```python
import functools
import math

import jax
import jax.numpy as jnp
from jax import lax
from jax.experimental import pallas as pl
from jax.experimental.pallas import tpu as pltpu

BF = jnp.bfloat16
F32 = jnp.float32
U32 = jnp.uint32
NT = (((1,), (1,)), ((), ()))


def _bf(x):
    return pltpu.bitcast(x, BF)


def _dot(a, b):
    return jnp.dot(a, b, preferred_element_type=F32)


def _ds(start, size, align):
    return pl.ds(start if isinstance(start, int) else pl.multiple_of(start, align), size)


def _run(jobs):
    for job in jobs:
        job()


def _part(jobs, k, first, end):
    if not first <= k < end:
        return []
    return jobs[(k - first) * len(jobs) // (end - first):(k + 1 - first) * len(jobs) // (end - first)]


_LHS = ((0, 1, 3), (2, 1, 3), (0,), (3,), (0, 1, 1), (2, -1, 0), (1, -1, 3))
_RHS = ((0, 1, 3), (0,), (1, -1, 3), (2, -1, 0), (3,), (0, 1, 1), (2, 1, 3))
_ORDER = (1, 3, 0, 2, 4, 5, 6)


def _operand(rule, block):
    if len(rule) == 1:
        return block(rule[0])
    a, b = block(rule[0]), block(rule[2])
    return a + b if rule[1] > 0 else a - b


def _operand_jobs(rules, get, put, rows):
    def job(r, p1):
        block = [_operand(rules[p1], lambda q1: get(2 * (q1 // 2) + q // 2, 2 * (q1 % 2) + q % 2, r).astype(F32))
                 for q in range(4)]
        for p2 in range(7):
            put(7 * p1 + p2, r, _operand(rules[p2], block.__getitem__).astype(BF))
    return [functools.partial(job, r, p1) for r in range(0, rows, 16) for p1 in range(7)]


def _combine(product, save, load, emit):
    def take(j, key, v):
        if j < 5:
            save(j, key, v)
        if j == 3:
            emit(2, key, load(1, key) + v)
        elif j == 4:
            emit(1, key, load(2, key) + v)
        elif j == 5:
            emit(3, key, (load(0, key) - load(1, key)) + (load(2, key) + v))
        elif j == 6:
            emit(0, key, (load(0, key) + load(3, key)) + (v - load(4, key)))
    for j in _ORDER:
        product(j, functools.partial(take, j))


def _strassen(product, shape, m_ref, zero, emit, side):
    rows, width = shape
    count = [0]

    def piece(n, r):
        return m_ref.at[zero + n, pl.ds(r % 128, 16), pl.ds((r // 128) * width, width)]

    def outer(j1, take1):
        base = 20 + 5 * (j1 % 2)

        def inner(j2, take2):
            res = product(7 * j1 + j2)
            for r in range(0, rows, 16):
                take2(r, res[r:r + 16])
            side(count[0])
            count[0] += 1

        def save(j, r, v):
            piece(base + j, r)[...] = v

        _combine(inner, save, lambda j, r: piece(base + j, r)[...], lambda q, r, v: take1((q, r), v))

    def save(j, key, v):
        piece(4 * j + key[0], key[1])[...] = v

    _combine(outer, save, lambda j, key: piece(4 * j + key[0], key[1])[...],
             lambda q1, key, v: emit(2 * (q1 // 2) + key[0] // 2, 2 * (q1 % 2) + key[0] % 2, key[1], v))


def _make_kernel(S, D, H, F):
    Dh = D // H
    TQ = 256
    CK = 128
    NC = S // CK
    NSTEP = (S // TQ) * H
    U = 16
    AHEAD = 4
    TM = 2 * TQ
    NB = S // TM
    R = TM // 4
    DK = D // 4
    HD = D // 2
    FC = 512
    NF = F // FC
    assert (D, Dh, NB, NF % 2, F) == (2 * FC, 32, 4, 1, NF * FC)
    qscale = (Dh ** -0.5) * math.log2(math.e)
    SEM_X, SEM_SMALL, SEM_DOWN, SEM_OUT = 4, 4 + NB, 7 + NB, 9 + NB

    def kernel(x_h, wq_h, wkt_h, wvt_h, wo_h, wg_h, wu_h, wd_h, gw_h, out_h,
               xa_v, ha_v, w_v, m_v, k_v, vt_v, g_v, ot_v, raw_v, rawd_v, zero_s, sem):
        @pl.loop(0, 3, unroll=False)
        def _(i):
            zero_s[0] = 2 - i

        def up_cp(c, slot):
            return [pltpu.make_async_copy(w_h.at[:, _ds(c * FC, FC, FC)], raw_v.at[slot, half], sem.at[2 * slot + half])
                    for half, w_h in enumerate((wg_h, wu_h))]

        def down_cp(c, slot):
            return pltpu.make_async_copy(wd_h.at[_ds(c * FC, FC, FC)], rawd_v.at[slot], sem.at[SEM_DOWN + slot])

        def up_jobs(slot, r0, rows):
            jobs = []
            for half in range(2):
                def put(p, r, v, half=half):
                    dst = w_v.at[p, _ds(slot * 128 + r0 // 2, rows // 2, 8)].bitcast(BF)
                    dst[pl.ds(r, 16), pl.ds(half * 128, 128)] = v
                jobs += _operand_jobs(_RHS, lambda a, b, r, half=half:
                                      raw_v[slot, half, _ds(r0 + a * DK + r, 16, 16), pl.ds(b * 128, 128)], put, rows)
            return jobs

        def wo_cp(slot, half):
            moves = ((0, 0, DK), (DK + 16, DK, HD - 16), (DK, DK + HD - 16, 16), (DK + HD, DK + HD, DK))
            return [pltpu.make_async_copy(wo_h.at[pl.ds(src, n), pl.ds(half * HD, HD)],
                                          raw_v.at[slot, half, pl.ds(dst, n)], sem.at[2 * slot + half])
                    for src, dst, n in moves]

        def o_row(unit):
            lo, hi = DK // 16, (DK + HD) // 16
            return jnp.where(unit == lo, hi - 1, jnp.where((unit > lo) & (unit < hi), unit - 1, unit))

        def anchor(i, p):
            return ha_v.at[i, 49], (p // 7) * 8, pl.ds((p % 7) * 128, 128)

        def project(qt_v, gt_v, x_v, wkv_v, gw_v):
            zero = zero_s[0]
            quarters = ((0, 0), (1, 0), (1, 1), (0, 1))
            wq_cp = [pltpu.make_async_copy(wq_h.at[pl.ds(a * HD, HD), pl.ds(b * HD, HD)],
                                           raw_v.at[1, b, pl.ds(a * HD, HD)], sem.at[2 * a + b]) for a, b in quarters]
            x0_cp = [pltpu.make_async_copy(x_h.at[rows, cols], x_v.at[rows, cols], sem.at[n]) for rows, cols, n in (
                (pl.ds(TQ, TQ), pl.ds(0, D), SEM_X), (pl.ds(0, TQ), pl.ds(0, HD), SEM_OUT),
                (pl.ds(0, TQ), pl.ds(HD, HD), SEM_DOWN))]

            def x_cp(i):
                return pltpu.make_async_copy(x_h.at[_ds(i * TM, TM, TM)], x_v.at[_ds(i * TM, TM, TM)], sem.at[SEM_X + i])

            small = [pltpu.make_async_copy(wkt_h, wkv_v.at[pl.ds(0, Dh)], sem.at[SEM_SMALL]),
                     pltpu.make_async_copy(wvt_h, wkv_v.at[pl.ds(Dh, Dh)], sem.at[SEM_SMALL + 1]),
                     pltpu.make_async_copy(gw_h, gw_v, sem.at[SEM_SMALL + 2])]

            def keys_values_gate(i):
                t = lax.dot_general(wkv_v[...], x_v[_ds(i * TM, TM, TM), :], NT, preferred_element_type=F32)
                g = jax.nn.sigmoid(t[2 * Dh:2 * Dh + 1])
                vt_v.bitcast(BF)[:, _ds(i * TM, TM, TM)] = t[Dh:2 * Dh].astype(BF)
                kg = jnp.concatenate([t[:Dh], jnp.broadcast_to(g, (128 - Dh, TM))], axis=0).T
                k_v[_ds(i * (TM // 2), TM // 2, TM // 2), :] = pltpu.bitcast(kg[:, :Dh].astype(BF), U32)
                g_v[_ds(i * TM, TM, TM), :] = jnp.broadcast_to(1.0 - kg[:, 127:128], (TM, 128))
                for a in range(2):
                    gt_v[2 * i + a] = g[:, a * TQ:(a + 1) * TQ]

            def x_jobs(i):
                def put(p, r, v):
                    cols = _ds(zero * 128, DK, 128) if isinstance(i, int) else pl.ds(0, DK)
                    xa_v.at[i, p].bitcast(BF)[pl.ds(r, 16), cols] = v
                    if r == 0:
                        ref, row, col = anchor(i, p)
                        ref.bitcast(BF)[pl.ds(2 * row, 16), col] = v[:, :128]
                return _operand_jobs(_LHS, lambda a, b, r: x_v[_ds(i * TM + a * R + r, 16, 16), pl.ds(b * DK, DK)], put, R)

            def wq_transposes(n):
                def job(r, c):
                    a, b = quarters[n]
                    dst = ot_v.at[zero + (b * HD + c) // DK].bitcast(BF)
                    dst[pl.ds((a * HD + r) // DK * DK + c % DK, 128), pl.ds(r % DK, 128)] = (
                        raw_v[1, b, pl.ds(a * HD + r, 128), pl.ds(c, 128)].T)
                return [functools.partial(job, r, c) for c in range(0, HD, 128) for r in range(0, HD, 128)]

            wq_jobs = []
            for c in range(0, DK, 128):
                def put_wq(p, r, v, c=c):
                    w_v.at[p, pl.ds(128, 128)].bitcast(BF)[pl.ds(r, 16), pl.ds(c, 128)] = v
                wq_jobs += _operand_jobs(_RHS, lambda a, b, r, c=c:
                                         _bf(ot_v[b, pl.ds((a * DK + r) // 2, 8), pl.ds(c, 128)]), put_wq, DK)

            def queries(i, side):
                after = i + 1 if isinstance(i, int) else jnp.minimum(i + 1, NB - 1)
                groups = [x_jobs(i)[j::7] for j in _ORDER[1:]] + [x_jobs(after)[_ORDER[0]::7]]

                def product(p):
                    w = w_v[p, pl.ds(128, 128), :]
                    if isinstance(i, int):
                        w = jnp.concatenate([w_v[p, pl.ds(128, 8), _ds(zero * 128, DK, 128)], w[8:]], axis=0)
                    return lax.dot_general(_bf(w), _bf(xa_v[i, p]), NT, preferred_element_type=F32)

                def emit(a, b, r, v):
                    dst = qt_v.at[(2 * i + a // 2) * H + (b * DK + r) // Dh].bitcast(BF)
                    dst[pl.ds(r % Dh, 16), pl.ds((a % 2) * R, R)] = (v * qscale).astype(BF)

                _strassen(product, (DK, R), m_v, zero, emit, lambda k: side(k, groups[k // 7]))

            _run([cp.start for cp in (wq_cp[0], x0_cp[0], wq_cp[1])])
            wq_cp[0].wait()
            _run([cp.start for cp in (wq_cp[2], x0_cp[1])])
            _run(wq_transposes(0) + wq_jobs[_ORDER[0]::7])
            x0_cp[0].wait()
            _run(x_jobs(0)[_ORDER[0]::7])
            arrivals = ((5, [wq_cp[3], x0_cp[2]], [wq_cp[1]]),
                        (9, small, [wq_cp[2], x0_cp[1]]),
                        (14, [x_cp(1)], [wq_cp[3], x0_cp[2]] + small))

            def first(k, x_group):
                n = k // 7
                w_first = x_first = 7 * n
                if n < 3:
                    at, start, wait = arrivals[n]
                    if k == at:
                        _run([cp.start for cp in start] + [cp.wait for cp in wait] + wq_transposes(n + 1))
                    w_first, x_first = at + 1, at if n == 1 else x_first
                if n < 6:
                    _run(_part(wq_jobs[_ORDER[n + 1]::7], k, w_first, 7 * n + 7) + _part(x_group, k, x_first, 7 * n + 7))
                if k == 15:
                    gw = gw_v[...].astype(F32)
                    gw_row = jnp.concatenate([gw[r:r + 1, :] for r in range(D // 128)], axis=1)
                    wkv_v[pl.ds(2 * Dh, 16), :] = jnp.broadcast_to(gw_row, (16, D)).astype(BF)
                    keys_values_gate(0)
                if k == 34:
                    x_cp(2).start()
                    x_cp(1).wait()
                if n == 6:
                    _run(_part(x_group, k, 42, 49))

            queries(0, first)

            @pl.loop(1, NB)
            def _(i):
                @pl.when(i == 1)
                def _():
                    x_cp(3).start()

                @pl.when(i == 2)
                def _():
                    _run([cp.start for cp in up_cp(0, 0) + up_cp(1, 1) + [down_cp(0, 0)]])

                @pl.when(i + 1 < NB)
                def _():
                    x_cp(i + 1).wait()

                def side(k, x_group):
                    _run(_part(x_group, k % 7, 0, 7))
                    if k == 0:
                        keys_values_gate(i)

                queries(i, side)

        def attend(qt_v, gt_v, s_v, o_v):
            def scores(n, slot, c, m8):
                s = _dot(_bf(k_v[pl.ds(c * CK // 2, CK // 2), :]), _bf(qt_v[n]))
                s_v[slot, pl.ds(c * CK, CK), :] = s
                for i in range(CK // 8):
                    t = s[i * 8:(i + 1) * 8]
                    m8[i % 2] = t if m8[i % 2] is None else jnp.maximum(m8[i % 2], t)

            def final_max(m8):
                m = jnp.max(jnp.maximum(m8[0], m8[1]), axis=0, keepdims=True)
                m8[0] = m8[1] = None
                return m

            def body(it, carry):
                m_max, m8 = carry
                m8 = list(m8)
                g = gt_v[it * U // H]
                jobs = up_jobs(0, it * (DK * U // NSTEP), DK * U // NSTEP)
                for j in range(U):
                    n = it * U + j
                    cur = j % 2
                    m = jnp.broadcast_to(m_max, (8, TQ))
                    l8 = [None, None]
                    for c in range(NC):
                        if c + AHEAD < NC:
                            scores(jnp.minimum(n + 1, NSTEP - 1), 1 - cur, c + AHEAD, m8)
                            if c + AHEAD == NC - 1:
                                m_max = final_max(m8)
                        else:
                            scores(jnp.minimum(n + 2, NSTEP - 1), cur, c + AHEAD - NC, m8)
                        p = jnp.exp2(s_v[cur, pl.ds(c * CK, CK), :].reshape(CK // 8, 8, TQ) - m[None])
                        for i in range(CK // 8):
                            l8[i % 2] = p[i] if l8[i % 2] is None else l8[i % 2] + p[i]
                        o = _dot(_bf(vt_v[:, pl.ds(c * CK, CK)]), p.reshape(CK, TQ).astype(BF))
                        if c > 0:
                            o = o_v[...] + o
                        if c < NC - 1:
                            o_v[...] = o
                    _run(_part(jobs, j, 0, U))
                    o = o * (g / jnp.sum(l8[0] + l8[1], axis=0, keepdims=True))
                    for part in range(2):
                        dst = ot_v.at[n // H, _ds(8 * o_row(2 * (n % H) + part), 8, 8)].bitcast(BF)
                        dst[...] = o[16 * part:16 * part + 16].astype(BF)
                return m_max, tuple(m8)

            m8 = [None, None]
            for c in range(NC):
                scores(0, 0, c, m8)
            m_max = final_max(m8)
            for c in range(AHEAD):
                scores(1, 1, c, m8)
            lax.fori_loop(0, NSTEP // U, body, (m_max, tuple(m8)))

        def attention(qt_v, gt_v):
            pl.run_scoped(functools.partial(project, qt_v, gt_v), pltpu.VMEM((S, D), BF),
                          pltpu.VMEM((2 * Dh + 16, D), BF), pltpu.VMEM((D // 128, 128), BF))
            _run([cp.wait for cp in up_cp(0, 0)])
            pl.run_scoped(functools.partial(attend, qt_v, gt_v), pltpu.VMEM((2, S, TQ), F32), pltpu.VMEM((Dh, TQ), F32))

        pl.run_scoped(attention, pltpu.VMEM((NSTEP, Dh // 2, TQ), U32), pltpu.VMEM((S // TQ, 1, TQ), F32))

        def ffn(h0_v, h1_v, on_v):
            h_v = (h0_v, h1_v)

            def down_jobs(c, slot, r0, rows):
                jobs = []
                for half in range(2):
                    def put(p, r, v, half=half):
                        dst = w_v.at[p, _ds(256 + c * 64 + r0 // 2, rows // 2, 8)].bitcast(BF)
                        dst[pl.ds(r, 16), pl.ds(half * 128, 128)] = v
                    jobs += _operand_jobs(_RHS, lambda a, b, r, half=half:
                                          rawd_v[slot, _ds(r0 + a * 128 + r, 16, 16), pl.ds(half * HD + b * 128, 128)],
                                          put, rows)
                return jobs

            def h_jobs(n, src, zero):
                def put(p, r, v):
                    ha_v.at[n % NB, p].bitcast(BF)[pl.ds(r, 16), _ds((n // NB) * 128, 128, 128)] = v
                return _operand_jobs(_LHS, lambda a, b, r: src[zero, 4 * a + b, pl.ds(r, 16), :], put, R)

            def o_jobs(i, r0, rows, zero):
                def put(p, r, v):
                    dst = ha_v.at[i, p, _ds(r0 // 2, rows // 2, 8)].bitcast(BF)
                    dst[pl.ds(r, 16), _ds((NF + zero) * 128, DK, 128)] = v
                return _operand_jobs(_LHS, lambda a, b, r:
                                     _bf(on_v[2 * i + a // 2, _ds(((a % 2) * R + r0 + r) // 2, 8, 8), pl.ds(b * DK, DK)]),
                                     put, rows)

            def o_transpose(tile, c):
                on_v.at[tile].bitcast(BF)[:, _ds(c * 128, 128, 128)] = _bf(ot_v[tile, _ds(c * 64, 64, 64), :]).T

            h1_v[...] = jnp.zeros(h1_v.shape, F32)
            on_v[:2] = jnp.zeros((2,) + on_v.shape[1:], U32)

            @pl.loop(0, 2 * NF)
            def _(t):
                c, half = t // 2, t % 2
                slot = c % 2
                zero = zero_s[0]

                @pl.when(half == 0)
                def _():
                    _run([cp.wait for cp in up_cp(0, 1 - slot)])

                    @pl.when(c + 1 < NF)
                    def _():
                        down_cp(c + 1, 1 - slot).start()

                    @pl.when(c + 2 == NF)
                    def _():
                        _run([cp.start for n in range(2) for cp in wo_cp(slot, n)])

                    @pl.when(c + 2 < NF)
                    def _():
                        _run([cp.start for cp in up_cp(c + 2, slot)])

                    down_cp(c, slot).wait()

                weights = up_jobs(1 - slot, half * (DK // 2), DK // 2) + down_jobs(c, slot, half * 64, 64)
                early = [functools.partial(o_transpose, c % 4, 4 * half + n) for n in range(4)]
                early += o_jobs(0, (t % (R // 16)) * 16, 16, zero)
                for u in range(2):
                    i = 2 * half + u
                    before = h_jobs(jnp.maximum(2 * t + u - 1, 0), h_v[1 - u], zero)

                    def product(p):
                        ref, row, col = anchor(i, p)
                        x = [xa_v[i, p, pl.ds(r, 8), :] for r in range(0, R // 2, 8)]
                        x[0] = jnp.concatenate([ref[pl.ds(row, 8), col], xa_v[i, p, pl.ds(0, 8), 128:]], axis=1)
                        return _dot(_bf(jnp.concatenate(x, axis=0)), _bf(w_v[p, _ds(slot * 128, 128, 128), :]))

                    def emit(a, b, r, v):
                        h_v[u][0, 4 * a + b, pl.ds(r, 16), :] = (
                            jnp.maximum(v[:, :128], 0.0) * v[:, 128:] * g_v[_ds(i * TM + a * R + r, 16, 8), :])

                    _strassen(product, (R, 256), m_v, zero, emit,
                              lambda k: _run(_part(early, 49 * u + k, 77, 91) + _part(_part(weights, u, 0, 2), k, 0, 49)
                                             + _part(before, k, 2, 35)))

            _run(h_jobs(NB * NF - 1, h1_v, 0))

            @pl.loop(0, 2 * NB)
            def _(t):
                i, half = t // 2, t % 2
                cols = _ds(half * 128, 128, 128)
                jobs = o_jobs(jnp.minimum(i + 1, NB - 1), half * (R // 2), R // 2, 0)
                jobs += [functools.partial(o_transpose, jnp.minimum(t + 4, 2 * NB - 1), c) for c in range(D // 128)]

                def out_cp(q):
                    return pltpu.make_async_copy(
                        raw_v.at[i // 2, i % 2, _ds(half * TM + (q // 2) * TQ, TQ, TQ), pl.ds((q % 2) * DK, DK)],
                        out_h.at[_ds(i * TM + (q // 2) * TQ, TQ, TQ), _ds(half * HD + (q % 2) * DK, DK, DK)],
                        sem.at[SEM_OUT])

                def product(p):
                    w = jnp.concatenate([_bf(w_v[p, pl.ds(256, NF * 64), cols]), _bf(w_v[p, pl.ds(128, 128), cols])], axis=0)
                    return _dot(_bf(ha_v[i, p]), w)

                def emit(a, b, r, v):
                    raw_v[i // 2, i % 2, _ds(half * TM + a * R + r, 16, 16), pl.ds(b * 128, 128)] = v.astype(BF)

                def side(k):
                    _run(_part(jobs, k, 0, 42))
                    if k == 42:
                        _run([out_cp(q).start for q in (2, 1, 3)])

                _strassen(product, (R, 128), m_v, zero_s[0], emit, side)
                out_cp(0).start()

            pltpu.make_async_copy(raw_v, raw_v, sem.at[SEM_OUT]).wait()

        pl.run_scoped(ffn, pltpu.VMEM((1, 16, R, 128), F32), pltpu.VMEM((1, 16, R, 128), F32),
                      pltpu.VMEM((S // TQ, TQ // 2, D), U32))

    scratch = [
        pltpu.VMEM((NB, 49, R // 2, DK), U32),
        pltpu.VMEM((NB, 50, R // 2, NF * 128 + DK), U32),
        pltpu.VMEM((49, 256 + NF * 64, 256), U32),
        pltpu.VMEM((30, 128, 256), F32),
        pltpu.VMEM((S // 2, Dh), U32),
        pltpu.VMEM((Dh // 2, S), U32),
        pltpu.VMEM((S, 128), F32),
        pltpu.VMEM((S // TQ, D // 2, TQ), U32),
        pltpu.VMEM((2, 2, D, FC), BF),
        pltpu.VMEM((2, FC, D), BF),
        pltpu.SMEM((1,), jnp.int32),
        pltpu.SemaphoreType.DMA((SEM_OUT + 1,)),
    ]
    return kernel, scratch


@jax.jit
def pallas_gated_mix__grouped_kv_mqa__glu_gated_reglu__prompt_kernel(
    A_x: jax.Array,
    A_wq: jax.Array,
    A_wk: jax.Array,
    A_wv: jax.Array,
    A_wo: jax.Array,
    B_x: jax.Array,
    B_W_gate: jax.Array,
    B_W_up: jax.Array,
    B_W_down: jax.Array,
    gate_w: jax.Array,
):
    del B_x
    B, S, D = A_x.shape
    kernel, scratch = _make_kernel(S, D, D // A_wk.shape[1], B_W_gate.shape[1])
    out = pl.pallas_call(
        kernel,
        out_shape=jax.ShapeDtypeStruct((S, D), A_x.dtype),
        in_specs=[pl.BlockSpec(memory_space=pl.ANY)] * 9,
        out_specs=pl.BlockSpec(memory_space=pl.ANY),
        scratch_shapes=scratch,
        compiler_params=pltpu.CompilerParams(vmem_limit_bytes=128 * 2 ** 20, disable_bounds_checks=True),
        name="fused",
    )(A_x.reshape(S, D), A_wq, A_wk.T, A_wv.T, A_wo, B_W_gate, B_W_up, B_W_down, gate_w.reshape(D // 128, 128))
    return out.reshape(B, S, D)
```
